```python
import os as _os
_os.environ.setdefault("JAX_PLATFORMS", "cpu")
import jax
import jax.numpy as jnp

def _softmax(x, axis=-1):
    return jax.nn.softmax(x, axis=axis)
def _gelu(x):
    return jax.nn.gelu(x, approximate=True)
def _silu(x):
    return jax.nn.silu(x)
def _sigmoid(x):
    return jax.nn.sigmoid(x)
def _layernorm(x, axis=-1, eps=1e-5):
    m = jnp.mean(x, axis=axis, keepdims=True)
    v = jnp.var(x, axis=axis, keepdims=True)
    return (x - m) / jnp.sqrt(v + eps)
def _scatter_add(tgt, idx, src, axis=0):
    return tgt.at[idx].add(src)
def _segment_sum(src, seg, n):
    return jax.ops.segment_sum(src, seg, n)
class _Rng:
    def __init__(self, key):
        self._k = key
    def _next(self):
        self._k, sub = jax.random.split(self._k)
        return sub
    def normal(self, shape):
        return jax.random.normal(self._next(), shape, dtype=jnp.bfloat16)
    def randint(self, lo, hi, shape):
        return jax.random.randint(self._next(), shape, lo, hi, dtype=jnp.int32)
    def uniform(self, shape, lo=0.0, hi=1.0):
        return jax.random.uniform(self._next(), shape, jnp.bfloat16, lo, hi)
    def permutation(self, n):
        return jax.random.permutation(self._next(), n)


kernel_name = 'standalone__gqa_softmax__near_ridge'

def setup_inputs():
    _rng = _Rng(jax.random.key(int.from_bytes(__import__("os").urandom(4), "little")))
    _w = (lambda a: (lambda t: t.astype(jnp.bfloat16) if jnp.issubdtype(t.dtype, jnp.floating) else t)(jnp.asarray(a)))
    B, Hq, Hkv, Sq, Sk, D = 8, 16, 8, 512, 512, 256
    return {
        "q": _w((lambda *s: _rng.normal(s) * 0.4)(B, Hq, Sq, D)),
        "k": _w((lambda *s: _rng.normal(s) * 0.4)(B, Hkv, Sk, D)),
        "v": _w((lambda *s: _rng.normal(s) * 0.05)(B, Hkv, Sk, D)),
    }

def reference(q, k, v):
    B, Hq, Sq, D = q.shape
    Hkv = k.shape[1]
    rep = Hq // Hkv
    k = jnp.repeat(k, rep, axis=1)
    v = jnp.repeat(v, rep, axis=1)
    scale = D ** -0.5
    scores = jnp.einsum("bhqd,bhkd->bhqk", q, k) * scale
    p = _softmax(scores, axis=-1)
    return jnp.einsum("bhqk,bhkd->bhqd", p, v)
```

```python
import jax
import jax.numpy as jnp
import jax.experimental.pallas as pl
import jax.experimental.pallas.tpu as pltpu

LOG2E = 1.4426950408889634

ROWS = 128
LAG = 2
UNROLL = 16
PREFETCH = 4
FIRST_LOADS = ("k", (0, 1), (1, 3), "v", (3, 4), (4, 6), (6, 8))
LAST_STORES = ((0, 4), (4, 6), (6, 7), (7, 8))


def _attention_kernel(q_hbm, k_hbm, v_hbm, o_hbm,
                      q_buf, k_buf, v_buf, o_buf, load_sems, store_sem):
    n_groups, group_rows, head_dim = q_buf.shape
    n_units = group_rows // ROWS
    n_iters = n_groups // UNROLL
    exp2_scale = head_dim ** -0.5 * LOG2E

    def unit_rows(lo, hi):
        return pl.ds(lo * ROWS, (hi - lo) * ROWS)

    def load_pieces(g, j):
        if j:
            return [(("qk", 0), src, dst, g, len(FIRST_LOADS) + j - 1)
                    for src, dst in ((k_hbm, k_buf), (q_hbm, q_buf), (v_hbm, v_buf))]
        pieces = []
        for sem, piece in enumerate(FIRST_LOADS):
            if piece == "k":
                pieces.append((("qk", 0), k_hbm, k_buf, g, sem))
            elif piece == "v":
                pieces.append((("pv", 0), v_hbm, v_buf, g, sem))
            else:
                pieces.append(
                    (("qk", piece[0]), q_hbm, q_buf, (g, unit_rows(*piece)), sem))
        return pieces

    def start_loads(g, j):
        for _, src, dst, idx, sem in load_pieces(g, j):
            pltpu.make_async_copy(src.at[idx], dst.at[idx], load_sems.at[sem]).start()

    def wait_loads(g, j, consumer):
        for who, src, dst, idx, sem in load_pieces(g, j):
            if who == consumer:
                pltpu.make_async_copy(src.at[idx], dst.at[idx], load_sems.at[sem]).wait()

    def iteration(it, carry):
        def scores(j, u):
            g = it * UNROLL + j
            wait_loads(g, j, ("qk", u))
            if u == 1:
                ahead = j + PREFETCH
                if ahead < UNROLL:
                    start_loads(g + PREFETCH, ahead)
                else:
                    @pl.when(it + 1 < n_iters)
                    def _():
                        start_loads(g + PREFETCH, ahead - UNROLL)
            return jax.lax.dot_general(
                q_buf[g, u * ROWS:(u + 1) * ROWS, :], k_buf[g],
                (((1,), (1,)), ((), ())), preferred_element_type=jnp.float32)

        def attend(j, u, s):
            g = it * UNROLL + j
            p = jnp.exp2((s - jnp.max(s, axis=-1, keepdims=True)) * exp2_scale)
            denom = jnp.sum(p, axis=-1, keepdims=True)
            inv = pl.reciprocal(denom, approx=True)
            inv = inv * (2.0 - denom * inv)
            p = (p * inv).astype(v_buf.dtype)
            wait_loads(g, j, ("pv", u))
            o = jnp.dot(p, v_buf[g], preferred_element_type=jnp.float32)
            o_buf[g, u * ROWS:(u + 1) * ROWS, :] = o.astype(o_buf.dtype)
            for lo, hi in LAST_STORES if j == UNROLL - 1 else ((0, n_units),):
                if hi == u + 1:
                    rows = unit_rows(lo, hi)
                    pltpu.make_async_copy(
                        o_buf.at[g, rows], o_hbm.at[g, rows], store_sem).start()

        units = [(j, u) for j in range(UNROLL) for u in range(n_units)]
        pending = []
        for t in range(len(units) + LAG):
            if t < len(units):
                pending.append(scores(*units[t]))
            if t >= LAG:
                attend(*units[t - LAG], pending.pop(0))
        return carry

    for g in range(PREFETCH):
        start_loads(g, g)
    jax.lax.fori_loop(0, n_iters, iteration, 0)
    pltpu.make_async_copy(o_buf, o_hbm, store_sem).wait()


@jax.jit
def pallas_standalone__gqa_softmax__near_ridge_kernel(
    q: jax.Array,
    k: jax.Array,
    v: jax.Array,
):
    B, Hq, Sq, D = q.shape
    _, Hkv, Sk, _ = k.shape
    n_groups, group_rows = B * Hkv, (Hq // Hkv) * Sq
    assert n_groups % UNROLL == 0 and group_rows == LAST_STORES[-1][1] * ROWS

    q_shape, kv_shape = (n_groups, group_rows, D), (n_groups, Sk, D)
    out = pl.pallas_call(
        _attention_kernel,
        in_specs=[pl.BlockSpec(memory_space=pl.ANY)] * 3,
        out_specs=pl.BlockSpec(memory_space=pl.ANY),
        out_shape=jax.ShapeDtypeStruct(q_shape, q.dtype),
        scratch_shapes=[
            pltpu.VMEM(q_shape, q.dtype),
            pltpu.VMEM(kv_shape, k.dtype),
            pltpu.VMEM(kv_shape, v.dtype),
            pltpu.VMEM(q_shape, q.dtype),
            pltpu.SemaphoreType.DMA((len(FIRST_LOADS) + UNROLL - 1,)),
            pltpu.SemaphoreType.DMA(()),
        ],
        compiler_params=pltpu.CompilerParams(
            vmem_limit_bytes=110 * 1024 * 1024,
            disable_bounds_checks=True,
            disable_semaphore_checks=True,
            flags={"XLA_TPU_RESCHEDULE_DMA_DONES": True},
        ),
        name="gqa_attn",
    )(q.reshape(q_shape), k.reshape(kv_shape), v.reshape(kv_shape))
    return out.reshape(B, Hq, Sq, D)
```

```python
import jax
import jax.numpy as jnp
import jax.experimental.pallas as pl
import jax.experimental.pallas.tpu as pltpu

LOG2E = 1.4426950408889634

ROWS = 128
LAG = 3
UNROLL = 16
PREFETCH = 4
LEAD_LOADS = (
    ("k", (0, 1), (1, 2), (2, 4), "v", (4, 5), (5, 8)),
    ("k", (0, 2), "v", (2, 8)),
)
LAST_STORES = ((0, 4), (4, 6), (6, 7), (7, 8))


def _load_plan(j, n_units):
    sem = sum(len(pieces) for pieces in LEAD_LOADS[:j])
    if j >= len(LEAD_LOADS):
        return [(name, 0, n_units, sem + j - len(LEAD_LOADS)) for name in "kqv"]
    return [(piece, 0, n_units, sem + n) if piece in ("k", "v") else ("q", *piece, sem + n)
            for n, piece in enumerate(LEAD_LOADS[j])]


def _attention_kernel(q_hbm, k_hbm, v_hbm, o_hbm,
                      q_buf, k_buf, v_buf, o_buf, load_sems, store_sem):
    n_groups, group_rows, head_dim = q_buf.shape
    n_units = group_rows // ROWS
    n_iters = n_groups // UNROLL
    exp2_scale = head_dim ** -0.5 * LOG2E

    def unit_rows(lo, hi):
        return pl.ds(lo * ROWS, (hi - lo) * ROWS)

    def load(g, name, lo, hi, sem):
        if name == "q":
            rows = unit_rows(lo, hi)
            src, dst = q_hbm.at[g, rows], q_buf.at[g, rows]
        elif name == "k":
            src, dst = k_hbm.at[g], k_buf.at[g]
        else:
            src, dst = v_hbm.at[g], v_buf.at[g]
        return pltpu.make_async_copy(src, dst, load_sems.at[sem])

    def start_loads(g, j):
        for piece in _load_plan(j, n_units):
            load(g, *piece).start()

    def wait_loads(g, j, u, for_values):
        for name, lo, hi, sem in _load_plan(j, n_units):
            late = name == "v" and j < len(LEAD_LOADS)
            if lo == u and late == for_values:
                load(g, name, lo, hi, sem).wait()

    def iteration(it, carry):
        def scores(j, u):
            g = it * UNROLL + j
            wait_loads(g, j, u, for_values=False)
            if u == LAG:
                ahead = j + PREFETCH
                if ahead < UNROLL:
                    start_loads(g + PREFETCH, ahead)
                else:
                    @pl.when(it + 1 < n_iters)
                    def _():
                        start_loads(g + PREFETCH, ahead - UNROLL)
            return jax.lax.dot_general(
                q_buf[g, u * ROWS:(u + 1) * ROWS, :], k_buf[g],
                (((1,), (1,)), ((), ())), preferred_element_type=jnp.float32)

        def attend(j, u, s):
            g = it * UNROLL + j
            p = jnp.exp2((s - jnp.max(s, axis=-1, keepdims=True)) * exp2_scale)
            inv = pltpu.reciprocal(jnp.sum(p, axis=-1, keepdims=True), full_range=False)
            p = (p * inv).astype(v_buf.dtype)
            wait_loads(g, j, u, for_values=True)
            o = jnp.dot(p, v_buf[g], preferred_element_type=jnp.float32)
            o_buf[g, u * ROWS:(u + 1) * ROWS, :] = o.astype(o_buf.dtype)
            for lo, hi in LAST_STORES if j == UNROLL - 1 else ((0, n_units),):
                if hi == u + 1:
                    rows = unit_rows(lo, hi)
                    pltpu.make_async_copy(
                        o_buf.at[g, rows], o_hbm.at[g, rows], store_sem).start()

        units = [(j, u) for j in range(UNROLL) for u in range(n_units)]
        pending = []
        for t in range(len(units) + LAG):
            if t < len(units):
                pending.append(scores(*units[t]))
            if t >= LAG:
                attend(*units[t - LAG], pending.pop(0))
        return carry

    for g in range(PREFETCH):
        start_loads(g, g)
    jax.lax.fori_loop(0, n_iters, iteration, 0)
    pltpu.make_async_copy(o_buf, o_hbm, store_sem).wait()


@jax.jit
def pallas_standalone__gqa_softmax__near_ridge_kernel(
    q: jax.Array,
    k: jax.Array,
    v: jax.Array,
):
    B, Hq, Sq, D = q.shape
    _, Hkv, Sk, _ = k.shape
    n_groups, group_rows = B * Hkv, (Hq // Hkv) * Sq
    assert n_groups % UNROLL == 0 and group_rows == LAST_STORES[-1][1] * ROWS
    n_load_sems = sum(len(pieces) - 1 for pieces in LEAD_LOADS) + UNROLL

    q_shape, kv_shape = (n_groups, group_rows, D), (n_groups, Sk, D)
    out = pl.pallas_call(
        _attention_kernel,
        in_specs=[pl.BlockSpec(memory_space=pl.ANY)] * 3,
        out_specs=pl.BlockSpec(memory_space=pl.ANY),
        out_shape=jax.ShapeDtypeStruct(q_shape, q.dtype),
        scratch_shapes=[
            pltpu.VMEM(q_shape, q.dtype),
            pltpu.VMEM(kv_shape, k.dtype),
            pltpu.VMEM(kv_shape, v.dtype),
            pltpu.VMEM(q_shape, q.dtype),
            pltpu.SemaphoreType.DMA((n_load_sems,)),
            pltpu.SemaphoreType.DMA(()),
        ],
        compiler_params=pltpu.CompilerParams(
            vmem_limit_bytes=110 * 1024 * 1024,
            disable_bounds_checks=True,
            disable_semaphore_checks=True,
            flags={"XLA_TPU_RESCHEDULE_DMA_DONES": True},
        ),
        name="gqa_attn",
    )(q.reshape(q_shape), k.reshape(kv_shape), v.reshape(kv_shape))
    return out.reshape(B, Hq, Sq, D)
```
